```python
import jax
import jax.numpy as jnp

def _softmax(x, axis=-1):
    return jax.nn.softmax(x, axis=axis)

def _gelu(x):
    return jax.nn.gelu(x, approximate=True)

def _silu(x):
    return jax.nn.silu(x)

def _sigmoid(x):
    return jax.nn.sigmoid(x)

def _layernorm(x, axis=-1, eps=1e-05):
    m = jnp.mean(x, axis=axis, keepdims=True)
    v = jnp.var(x, axis=axis, keepdims=True)
    return (x - m) / jnp.sqrt(v + eps)

def _scatter_add(tgt, idx, src, axis=0):
    return tgt.at[idx].add(src)

def _segment_sum(src, seg, n):
    return jax.ops.segment_sum(src, seg, n)

class _Rng:

    def __init__(self, key):
        self._k = key

    def _next(self):
        self._k, sub = jax.random.split(self._k)
        return sub

    def normal(self, shape):
        return jax.random.normal(self._next(), shape, dtype=jnp.bfloat16)

    def randint(self, lo, hi, shape):
        return jax.random.randint(self._next(), shape, lo, hi, dtype=jnp.int32)

    def uniform(self, shape, lo=0.0, hi=1.0):
        return jax.random.uniform(self._next(), shape, jnp.bfloat16, lo, hi)

    def permutation(self, n):
        return jax.random.permutation(self._next(), n)
kernel_name = 'adaLN_cond__grouped_kv_mqa__mixer_token_mlp__prompt'

def _fwd_setup_inputs():
    _rng = _Rng(jax.random.key(int.from_bytes(__import__("os").urandom(4), "little")))
    _w = lambda a: (lambda t: t.astype(jnp.bfloat16) if jnp.issubdtype(t.dtype, jnp.floating) else t)(jnp.asarray(a))

    def _A_setup():
        B, S, D, H = (1, 2048, 512, 32)
        Dh = D // H
        return {'x': _w((lambda *s: _rng.normal(s) * 0.05)(B, S, D)), 'wq': _w((lambda *s: _rng.normal(s) * 0.05)(D, H * Dh)), 'wk': _w((lambda *s: _rng.normal(s) * 0.05)(D, Dh)), 'wv': _w((lambda *s: _rng.normal(s) * 0.05)(D, Dh)), 'wo': _w((lambda *s: _rng.normal(s) * 0.05)(H * Dh, D))}
    _A_in = _A_setup()

    def _B_setup():
        B, S, D, F = (1, 2048, 512, 1376)
        return {'x': _w((lambda *s: _rng.normal(s) * 0.05)(B, S, D)), 'w1': _w((lambda *s: _rng.normal(s) * 0.05)(S, F) * S ** (-0.5)), 'b1': _w((lambda *s: _rng.normal(s) * 0.05)(F) * 0.02), 'w2': _w((lambda *s: _rng.normal(s) * 0.05)(F, S) * F ** (-0.5)), 'b2': _w((lambda *s: _rng.normal(s) * 0.05)(S) * 0.02)}
    _B_in = _B_setup()
    return {'A_x': _A_in['x'], 'A_wq': _A_in['wq'], 'A_wk': _A_in['wk'], 'A_wv': _A_in['wv'], 'A_wo': _A_in['wo'], 'B_x': _B_in['x'], 'B_w1': _B_in['w1'], 'B_b1': _B_in['b1'], 'B_w2': _B_in['w2'], 'B_b2': _B_in['b2'], 'c': _w((lambda *s: _rng.normal(s) * 0.05)(1, 512)), 'w_mod': _w((lambda *s: _rng.normal(s) * 0.05)(512, 6 * 512) * 512 ** (-0.5))}

def _fwd_reference(A_x, A_wq, A_wk, A_wv, A_wo, B_x, B_w1, B_b1, B_w2, B_b2, c, w_mod):

    def _A_ref(x, wq, wk, wv, wo):
        B, S, D = x.shape
        H = 32
        Dh = D // H
        q = (lambda x, *d: x.transpose(*d))((x @ wq).reshape(B, S, H, Dh), 0, 2, 1, 3)
        k = x @ wk
        v = x @ wv
        scores = jnp.einsum('bhqd,bkd->bhqk', q, k) * Dh ** (-0.5)
        p = _softmax(scores, axis=-1)
        o = jnp.einsum('bhqk,bkd->bhqd', p, v)
        return (lambda x, *d: x.transpose(*d))(o, 0, 2, 1, 3).reshape(B, S, H * Dh) @ wo

    def _B_ref(x, w1, b1, w2, b2):
        B, S, D = x.shape
        h = _layernorm(x, axis=-1)
        u = jnp.einsum('bsd,sf->bdf', h, w1) + b1
        u = _gelu(u)
        y = jnp.einsum('bdf,fs->bds', u, w2) + b2
        return (lambda x, *d: x.transpose(*d))(y, 0, 2, 1)
    x = A_x
    mod = (_silu(c) @ w_mod).reshape(c.shape[0], 6, 1, -1)
    sa, ca, ga, sb, cb, gb = (mod[:, 0].copy(), mod[:, 1].copy(), mod[:, 2].copy(), mod[:, 3].copy(), mod[:, 4].copy(), mod[:, 5].copy())
    h = _layernorm(x, axis=-1) * (1 + ca) + sa
    x = x + ga * _A_ref(h, A_wq, A_wk, A_wv, A_wo)
    h = _layernorm(x, axis=-1) * (1 + cb) + sb
    x = x + gb * _B_ref(h, B_w1, B_b1, B_w2, B_b2)
    return x

def setup_inputs():
    _inp = _fwd_setup_inputs()
    _gk = jax.random.fold_in(jax.random.key(int.from_bytes(__import__("os").urandom(4), "little")), 2 ** 31 - 1)
    _shapes = [[1, 2048, 512]]
    _dtypes = ['bfloat16']
    _gks = jax.random.split(_gk, len(_shapes))
    _gs = [jax.random.normal(k, s, dtype=jnp.dtype(d)) * 0.05 for k, s, d in zip(_gks, _shapes, _dtypes)]
    _inp['grad_out'] = _gs[0]
    return _inp

def reference(A_x, A_wq, A_wk, A_wv, A_wo, B_w1, B_b1, B_w2, B_b2, c, w_mod, B_x, grad_out):
    _const = dict(B_x=B_x)

    def _f(*_d):
        return _fwd_reference(**{'A_x': _d[0], 'A_wq': _d[1], 'A_wk': _d[2], 'A_wv': _d[3], 'A_wo': _d[4], 'B_w1': _d[5], 'B_b1': _d[6], 'B_w2': _d[7], 'B_b2': _d[8], 'c': _d[9], 'w_mod': _d[10], **_const})
    _out, _vjp = jax.vjp(_f, A_x, A_wq, A_wk, A_wv, A_wo, B_w1, B_b1, B_w2, B_b2, c, w_mod)
    _grads = _vjp(grad_out)
    _out0 = jnp.asarray(_out)
    return (_out0, *[jnp.asarray(_g) for _g in _grads])
```

```python
import functools
import math

import jax
import jax.numpy as jnp
from jax import lax
import jax.experimental.pallas as pl
import jax.experimental.pallas.tpu as pltpu

bf16 = jnp.bfloat16
f32 = jnp.float32
i32 = jnp.int32

S, D, H, DH, F = 2048, 512, 32, 16, 1376
EPS = 1e-5
QB = 512
KC = 128
NC = S // KC
NBLK = H * (S // QB)
KEPT = (KC - 16) // 2
SLOT = NC * KEPT
NSLOT = 59
NSPILL = NBLK - NSLOT
NRING = NSLOT + 1
RING0 = (NSLOT - (NBLK - NRING)) % NRING
FBODY, BBODY = 4, 8
EARLY = 3
LATER = 16
MAX_GAP = 48.0
TC = 256
NTC = S // TC
FC = 128
NFC = F // FC
FREM = F - NFC * FC

QSCALE = DH ** -0.5 * math.log2(math.e)
NT = (((1,), (1,)), ((), ()))


def _pack(x):
    return pltpu.bitcast(x.astype(bf16), i32)


def _unpack(x):
    return pltpu.bitcast(x, bf16)


def _dot(a, b):
    return jnp.dot(a, b, preferred_element_type=f32)


def _dot_nt(a, b):
    return lax.dot_general(a, b, NT, preferred_element_type=f32)


def _chain(op, xs, init=None):
    for x in xs:
        init = x if init is None else op(init, x)
    return init


def _fold_lanes(x):
    return _chain(jnp.add, [x[:, j:j + 128] for j in range(0, x.shape[1], 128)])


def _col(row):
    return jnp.broadcast_to(row, (128, row.shape[1])).T


def _wide(col, n):
    return jnp.concatenate([col] * (n // 128), axis=1)


def _row_total(acc):
    return jnp.sum(acc.T, axis=0, keepdims=True)


def _paced(x, always, pace):
    return x if pace is None else jnp.where(_wide(always[:1], x.shape[1]), x, pace)


def _ln_stats(x, always=None, pace=None):
    d = x - x[0:1]
    m = jnp.mean(d, axis=0, keepdims=True)
    var = jnp.maximum(jnp.mean(d * d, axis=0, keepdims=True) - m * m, 0.0)
    r = lax.rsqrt(var + EPS)
    return x[0:1] + m, r, (_paced(d, always, pace) - m) * r


def _ln_bwd(dy, xhat, r, always=None, pace=None):
    a = jnp.mean(dy, axis=0, keepdims=True)
    b = jnp.mean(dy * xhat, axis=0, keepdims=True)
    return r * (_paced(dy, always, pace) - a - xhat * b)


def _ds(i, n):
    if isinstance(i, int):
        return pl.ds(i * n, n)
    return pl.ds(pl.multiple_of(i * n, n), n)


def _block(b):
    return _ds(b >> 2, 8), _ds(b & 3, QB)


def _token_major(x):
    return jnp.concatenate([x, jnp.zeros((128 - x.shape[0], x.shape[1]), f32)], axis=0).T


def _minus_rows(x):
    row = lax.broadcasted_iota(i32, (16, x.shape[1]), 0)
    hi = x.astype(bf16).astype(f32)
    mid = (x - hi).astype(bf16).astype(f32)
    lo = x - hi - mid
    return _pack(jnp.where(row == 0, -hi, jnp.where(row == 1, -mid, jnp.where(row == 2, -lo, 0.0))))


def _spread_lanes(table, n, rows):
    for i in range(DH):
        r0 = n % 2 * 256 + i * 16
        table[n // 2, r0:r0 + 16] = jnp.broadcast_to(rows[:, i:i + 1], (16, 128))


def _spread_sublanes(table, w16):
    w = w16.astype(f32)
    for i in range(DH):
        table[i * 8:(i + 1) * 8] = jnp.broadcast_to(w[i:i + 1], (8, QB))


def _vpu_dot(lhs, n, rhs, init, always):
    acc, marks = init, []
    for i in range(DH):
        r0 = n % 2 * 256 + i * 16
        b = rhs[i * 8:(i + 1) * 8, :]
        term = _wide(lhs[n // 2, r0:r0 + 16], QB) * jnp.concatenate([b, b], axis=0)
        acc = acc + term
        if i % 8 == 7:
            marks.append(jnp.where(_wide(always, QB), acc[:8], acc[8:]))
    return acc, [m[:, j:j + 128] for j in range(0, QB, 128) for m in marks]


def _after(words, token, always):
    if token is None:
        return words
    first = jnp.where(always, words[:, :128], pltpu.bitcast(token, i32))
    return first if words.shape[1] == 128 else jnp.concatenate([first, words[:, 128:]], axis=1)


def _kernel(
    c_hbm, b1_hbm, b2_hbm, wkT_hbm, wvT_hbm, x_hbm, wq_hbm, wo_hbm, w1T_hbm, w2_hbm, wmod_hbm,
    dout_hbm,
    dc_hbm, db1_hbm, db2_hbm, dwkT_hbm, dwvT_hbm, dx_hbm, dwq_hbm, dwo_hbm, dw1T_hbm, dw2_hbm,
    dwmod_hbm, out_hbm, spill_hbm,
    pool, qT, aux, kvT, linv, shift, stats, ltab, stab, keys, mod, dmod, zeros,
    wsq, wk, wv, b2, cv,
    b1, db1,
    one, psem, wsem, ssem,
):
    small_in = [pltpu.make_async_copy(src, dst, ssem.at[k]) for k, (src, dst) in
                enumerate(zip((c_hbm, b1_hbm, b2_hbm, wkT_hbm, wvT_hbm),
                              (cv, b1, b2, wk, wv)))]
    small_out = [pltpu.make_async_copy(src, dst, ssem.at[k]) for k, (src, dst) in
                 enumerate(zip((cv, db1, b2, wk, wv),
                               (dc_hbm, db1_hbm, db2_hbm, dwkT_hbm, dwvT_hbm)))]

    def silu_c(rows):
        c32 = cv[...].astype(f32)
        return jnp.broadcast_to(c32 * jax.nn.sigmoid(c32), (rows, D))

    zeros[...] = jnp.zeros_like(zeros)
    one[0] = 1

    def mod_grad(wm, dm):
        part = _dot_nt(jnp.broadcast_to(dm, (16, D)).astype(bf16), wm[...])[0:1]
        wm[...] = (_wide(silu_c(128).T, D) * dm).astype(bf16)
        return part

    def mod_copies(buf, sem, first):
        def load(k):
            return pltpu.make_async_copy(wmod_hbm.at[:, _ds(first + k, D)], buf.at[k], sem.at[k])

        def store(k):
            return pltpu.make_async_copy(buf.at[k], dwmod_hbm.at[:, _ds(first + k, D)], sem.at[k])

        return [load(k) for k in range(3)], store

    def pool_slot(slot):
        return pool.at[_ds(slot, SLOT)]

    def spill_copy(j, slot):
        return pltpu.make_async_copy(pool_slot(slot), spill_hbm.at[_ds(j, SLOT)], psem.at[slot])

    def fill_copy(j, count):
        slot = j + NSLOT - NSPILL
        return pltpu.make_async_copy(
            spill_hbm.at[pl.ds(_ds(j, SLOT).start, count * SLOT)],
            pool.at[pl.ds(_ds(slot % NSLOT if isinstance(j, int) else slot, SLOT).start,
                          count * SLOT)],
            psem.at[j % NRING])

    def panel(t, n):
        per = QB // n
        j = t // per
        start = NSLOT * SLOT + (j ^ 2) * D
        if not isinstance(start, int):
            start = pl.multiple_of(start, 8)
        return pl.ds(start, D), _ds(t % per, n)

    def load_panel(t, n):
        return pltpu.bitcast(pool[panel(t, n)], f32)

    def store_panel(t, n, x):
        pool[panel(t, n)] = pltpu.bitcast(x, i32)

    def key_groups(c, groups):
        return [keys[c * KC // 2 + g * 8:c * KC // 2 + g * 8 + 8, :] for g in groups]

    def key_lhs(words, width=DH):
        return _unpack(jnp.concatenate(words, axis=0))[:, :width]

    def region(fn):
        lax.fori_loop(0, one[0], lambda _, carry: (fn(), carry)[1], 0)

    def start_now(*copies):
        region(lambda: [cp.start() for cp in copies])

    wq_copy = pltpu.make_async_copy(wq_hbm, wsq, wsem)
    dwo_copy = pltpu.make_async_copy(wsq, dwo_hbm, wsem)

    def phase_main(oT, dob, late, sem, park_sem):
        cols, acc = ltab.at[4:8], ltab.at[0:3]
        cdo = pltpu.make_async_copy(dout_hbm, dob, sem)
        park = pltpu.make_async_copy(pool_slot(RING0), late.at[0:SLOT], psem.at[RING0])
        unpark = pltpu.make_async_copy(late.at[0:SLOT], spill_hbm.at[0:SLOT], park_sem)
        cwo = pltpu.make_async_copy(wo_hbm, dob.at[0:D], sem)

        def pass_attention(wmbuf, asem):
            cm = [pltpu.make_async_copy(wmod_hbm.at[:, j * 1024:(j + 1) * 1024], wmbuf.at[j % 2],
                                        asem.at[j]) for j in range(3)]
            cx = [pltpu.make_async_copy(x_hbm.at[j * QB:(j + 1) * QB], dob.at[j * QB:(j + 1) * QB],
                                        asem.at[3 + j]) for j in range(4)]
            cw = (*small_in, pltpu.make_async_copy(wq_hbm.at[:, :128], wsq.at[:, :128], asem.at[7]))
            cq = pltpu.make_async_copy(wq_hbm.at[:, 128:], wsq.at[:, 128:], asem.at[8])
            for cp in (cx[0], cx[1], cm[0], *cw):
                cp.start()
            hT = pool.at[pl.ds((RING0 - 2) * SLOT, S // 2)]
            affine, wqT = pool_slot(RING0 - 3), pool.at[pl.ds((RING0 - 4) * SLOT, 192)]

            def normed(j):
                xT = dob[_ds(j, QB)].T
                aux[:, _ds(j, QB)] = pltpu.bitcast(xT, i32)
                return _ln_stats(xT.astype(f32))[2]

            def store_q(rows, j, q):
                q16 = (q * QSCALE).astype(bf16)
                qT[rows.start * 8:rows.stop * 8, _ds(j, QB)] = pltpu.bitcast(q16, i32)
                sq = q16.astype(f32) * q16.astype(f32)
                shift[rows, _ds(j, QB)] = jnp.concatenate(
                    [jnp.sum(sq[r:r + DH], axis=0, keepdims=True)
                     for r in range(0, q.shape[0], DH)], axis=0)

            def project(j, xhat):
                h16 = (xhat * _wide(pltpu.bitcast(affine[0:D, 128:256], f32), QB)
                       + _wide(pltpu.bitcast(affine[0:D, 0:128], f32), QB)).astype(bf16)
                hT[_ds(j, D // 2)] = pltpu.bitcast(h16, i32)
                kvq = _dot(_unpack(stab[1, 0:80]), h16)
                kvT[:, _ds(j, QB)] = _pack(kvq[:2 * DH])
                store_q(slice(0, 8), j, kvq[2 * DH:])
                k = _token_major(jnp.concatenate(
                    [kvq[:DH].astype(bf16).astype(f32), jnp.ones((8, QB), f32)], axis=0))
                keys[_ds(j, QB // 2)] = _pack(k)
                for c in range(QB // KC):
                    _spread_lanes(ltab, j * (QB // KC) + c, k[(c + 1) * KC - 16:(c + 1) * KC])

            def choose_shift(rows):
                kmax, kmean = dmod[0:1, 0:1], dmod[1:2, 0:1]
                qnorm = jnp.sqrt(shift[rows])
                shift[rows] = qnorm * kmax
                unsafe = jnp.where(qnorm * (kmax + kmean) <= MAX_GAP, 0.0, 1.0)

                def row_max(b, _):
                    w = _unpack(qT[_block(b)])
                    mx = None
                    for c in range(NC):
                        sc = _dot(key_lhs(key_groups(c, range(8))), w)
                        mx = _chain(jnp.maximum, [sc[r:r + 8] for r in range(0, KC, 8)], mx)
                    shift[pl.ds(b >> 2, 1), _block(b)[1]] = jnp.max(mx, axis=0, keepdims=True)
                    return 0

                @pl.when(jnp.max(unsafe) > 0.0)
                def _():
                    lax.fori_loop(4 * rows.start, 4 * rows.stop, row_max, 0)

            cx[0].wait()
            store_panel(0, QB, normed(0))
            cx[1].wait()
            start_now(cx[2], cx[3])
            store_panel(1, QB, normed(1))
            for cp in (*cw, cm[0]):
                cp.wait()
            stab[1, 0:80] = pltpu.bitcast(
                jnp.concatenate([wk[...], wv[...], wsq[:, :128].T], axis=0), f32)
            m01 = _dot(silu_c(16).astype(bf16), wmbuf[0])[0:1]
            mod[0:1] = m01[:, :D]
            mod[1:2] = m01[:, D:]
            affine[0:D, 0:128] = pltpu.bitcast(_col(m01[:, :D]), i32)
            affine[0:D, 128:256] = pltpu.bitcast(_col(1.0 + m01[:, D:]), i32)
            project(0, load_panel(0, QB))
            project(1, load_panel(1, QB))
            cx[2].wait()
            cx[3].wait()
            start_now(cq, cm[1], cm[2])
            project(2, normed(2))
            project(3, normed(3))
            k32 = _unpack(kvT[0:8]).astype(f32)
            ksq = jnp.max(jnp.sum(k32 * k32, axis=0, keepdims=True), axis=1, keepdims=True)
            kbar = jnp.mean(k32, axis=1, keepdims=True)
            dmod[0:1, 0:1] = jnp.sqrt(ksq) * (1.0 + 2.0 ** -10)
            dmod[1:2, 0:1] = jnp.sqrt(jnp.sum(kbar * kbar, axis=0, keepdims=True))
            for i in range(2):
                _spread_sublanes(stab.at[i], _unpack(qT[_block(i)]))
            choose_shift(slice(0, 8))
            cwo.start()

            def later_setup():
                for cp in (cq, cm[1], cm[2], park):
                    cp.wait()
                wqT[...] = pltpu.bitcast(wsq[:, 128:].T, i32)

                def other_heads(j, _):
                    store_q(slice(8, H), j,
                            _dot(_unpack(wqT[...]), _unpack(hT[_ds(j, D // 2)])))
                    return 0

                lax.fori_loop(0, S // QB, other_heads, 0)
                for j in (1, 2):
                    mj = _dot(silu_c(16).astype(bf16), wmbuf[j % 2])[0:1]
                    mod[2 * j:2 * j + 1] = mj[:, :D]
                    mod[2 * j + 1:2 * j + 2] = mj[:, D:]
                choose_shift(slice(8, H))
                cwo.wait()
                wsq[...] = dob[0:D]

            def attend(b0, slots):
                always = zeros[...] == 0
                ctx = []
                for i in range(len(slots)):
                    b = b0 + i
                    m = shift[pl.ds(b >> 2, 1), _block(b)[1]]
                    ctx.append((m, jnp.concatenate([qT[_block(b)], _minus_rows(m)], axis=0)))
                vpu, p16, li = {}, {}, {}
                l = o = None
                n = len(slots) * NC
                for t in range(n + 2):
                    tok = [None] * 8
                    if t + 1 < n:
                        i, c = divmod(t + 1, NC)
                        vpu[t + 1], tok = _vpu_dot(ltab, c, stab.at[i % 2],
                                                   jnp.broadcast_to(-ctx[i][0], (16, QB)), always)
                    if t < n:
                        i, c = divmod(t, NC)
                        words = [_after(x, tk, always) for x, tk in
                                 zip(key_groups(c, range(7 if t > 0 else 8)),
                                     tok[:3] + tok[4:] + [None])]
                        sc = _dot(key_lhs(words, 2 * DH), _unpack(ctx[i][1]))
                        if t > 0:
                            sc = jnp.concatenate([sc, vpu.pop(t)], axis=0)
                        p = jnp.exp2(sc)
                        l = _chain(jnp.add, [p[r:r + 8] for r in range(0, KC, 8)],
                                   l if c > 0 else None)
                        p16[t] = p.astype(bf16)
                        slots[i][_ds(c, KEPT), :] = _pack(p[16:])
                        if c == NC - 1:
                            li[i] = 1.0 / jnp.sum(l, axis=0, keepdims=True)
                            ahead = jnp.minimum(b0 + i + 2, NBLK - 1)
                            _spread_sublanes(stab.at[i % 2], _unpack(qT[_block(ahead)]))
                    if t >= 2:
                        i, c = divmod(t - 2, NC)
                        r = _dot(_unpack(kvT[8:16, c * KC:(c + 1) * KC]), p16.pop(t - 2))
                        o = r if c == 0 else o + r
                        if c == NC - 1:
                            oT[_block(b0 + i)] = _pack(o * li[i])
                            linv[pl.ds((b0 + i) >> 2, 1), _block(b0 + i)[1]] = li[i]

            def fwd_steps(first, count, size, slot):
                def fwd_step(n, slot):
                    b0 = first + n * size
                    slots = [jnp.where(slot + i >= NRING, slot + i - NRING, slot + i)
                             for i in range(size + 1)]
                    for i in range(size):
                        @pl.when(b0 + i > NRING)
                        def _():
                            spill_copy(b0 + i - NRING, slots[i]).wait()

                    if size == FBODY:
                        pl.when(b0 == LATER)(later_setup)
                    else:
                        pl.when(b0 == 2)(park.start)
                    attend(b0, [pool_slot(x & 63) for x in slots[:size]])
                    for i in range(size):
                        @pl.when(jnp.logical_and(b0 + i > 0, b0 + i < NSPILL))
                        def _():
                            spill_copy(b0 + i, slots[i]).start()

                    return slots[size]

                return lax.fori_loop(0, count, fwd_step, slot)

            def fwd_phase(k, slot):
                slot = fwd_steps(k * (NBLK - FBODY), FBODY // 2, 2, slot)
                return fwd_steps(FBODY, (1 - k) * (NBLK // FBODY - 2), FBODY, slot)

            lax.fori_loop(0, 2, fwd_phase, RING0)

        pl.run_scoped(
            pass_attention, pltpu.VMEM((2, D, 1024), bf16),
            pltpu.SemaphoreType.DMA((9,)))

        def pass_mlp(early, osem):
            def store_early(f, k, words):
                early[k, :, _ds(f, FC)] = words

            def store_late(f, k, words):
                late[_ds(2 * k + ((f - EARLY) >> 2), D // 2), _ds((f - EARLY) & 3, FC)] = words

            def load_hidden(k):
                return _unpack(jnp.concatenate(
                    [early[k], late[_ds(2 * k, D // 2)], late[_ds(2 * k + 1, D // 2)]], axis=1))

            def weight_grads(g16, du16):
                d2 = _dot_nt(g16, dob[...]).astype(bf16)
                return _dot(du16, _unpack(aux[...])).astype(bf16), d2

            def pass_hidden(w1b, w2b, b1s, db1s, hsem):
                def cin(f, s, n=FC):
                    rows = pl.ds(pl.multiple_of(f * FC, FC), n)
                    return (pltpu.make_async_copy(w1T_hbm.at[rows], w1b.at[s, 0:n], hsem.at[0, s]),
                            pltpu.make_async_copy(w2_hbm.at[rows], w2b.at[s, 0:n], hsem.at[1, s]))

                def cout(f, s):
                    rows = _ds(f, FC)
                    return (pltpu.make_async_copy(w1b.at[s], dw1T_hbm.at[rows], hsem.at[0, s]),
                            pltpu.make_async_copy(w2b.at[s], dw2_hbm.at[rows], hsem.at[1, s]))

                start_now(*cin(0, 0), cdo)

                words = pltpu.bitcast(wsq[...].T, f32)
                stab[0], stab[1] = words[:128], words[128:]

                def normalize(half):
                    if half == 0:
                        for k, v in enumerate((mod[2:3], mod[3:4], 1.0 + mod[4:5], mod[5:6])):
                            cols[k] = _col(v)
                    always = zeros[...] == 0
                    woT = _unpack(jnp.concatenate([stab[0], stab[1]], axis=0))
                    chunks = [half * (NTC // 2) + k for k in range(NTC // 2)]
                    proj = [_dot(woT, _unpack(oT[:, _ds(t, TC)])) for t in chunks]
                    for t, a, following in zip(chunks, proj, proj[1:] + [None]):
                        ts = _ds(t, TC)
                        x1 = _unpack(aux[:, ts]).astype(f32) + _wide(cols[0], TC) * a
                        store_panel(t, TC, x1)
                        mu2, r2, xh2 = _ln_stats(x1)
                        mu3, r3, h3 = _ln_stats(xh2 * _wide(cols[2], TC) + _wide(cols[1], TC), always, following)
                        aux[:, ts] = _pack(h3)
                        for k, v in enumerate((mu2, r2, mu3, r3)):
                            stats[k:k + 1, ts] = v

                region(lambda: normalize(0))
                spill_copy(NSPILL - 1, NSLOT).wait()
                region(lambda: normalize(1))
                dmod[7:8] = jnp.zeros((1, D), f32)
                b1s[...] = jnp.zeros_like(b1s)
                b1s[:, 0:F] = b1[...].astype(f32).reshape(1, F)
                cdo.wait()
                unpark.start()

                def hidden(f, s, n, store):
                    fs = _ds(f, FC)
                    gb = mod[5:6]
                    u = _dot_nt(w1b[s, 0:n], _unpack(aux[...])) + _wide(_col(b1s[:, fs])[0:n], D)
                    dg = _dot(w2b[s, 0:n], dob[...])
                    k0 = math.sqrt(2.0 / math.pi)
                    u2 = u * u
                    th = jnp.tanh(u * (k0 + (k0 * 0.044715) * u2))
                    hp = 0.5 + 0.5 * th
                    g = u * hp
                    dmod[7:8] += jnp.sum(g * dg, axis=0, keepdims=True)
                    du = dg * gb * (hp + 0.5 * u * (1.0 - th * th) * (k0 + (3 * k0 * 0.044715) * u2))

                    def padded(v):
                        if n == FC:
                            return v
                        return jnp.concatenate([v, jnp.zeros((FC - n, v.shape[1]), f32)], axis=0)

                    for k, v in enumerate((g, du)):
                        store(f, k, pltpu.bitcast(padded(v).astype(bf16).T, i32))
                    db1s[:, fs] = _row_total(padded(_fold_lanes(du)))
                    return (g * gb).astype(bf16), du.astype(bf16)

                def body(store, f, s):
                    nxt = jnp.where(s == 2, 0, s + 1)

                    @pl.when(f >= 2)
                    def _():
                        for cp in cout(f - 2, nxt):
                            cp.wait()

                    @pl.when(f + 1 < NFC)
                    def _():
                        for cp in cin(f + 1, nxt):
                            cp.start()

                    @pl.when(f + 1 == NFC)
                    def _():
                        for cp in cin(f + 1, nxt, FREM):
                            cp.start()

                    for cp in cin(f, s):
                        cp.wait()
                    w1b[s], w2b[s] = weight_grads(*hidden(f, s, FC, store))
                    for cp in cout(f, s):
                        cp.start()
                    return nxt

                lax.fori_loop(0, EARLY, functools.partial(body, store_early), 0)
                unpark.wait()
                lax.fori_loop(EARLY, NFC, functools.partial(body, store_late), EARLY % 3)
                for cp in cin(NFC, NFC % 3, FREM):
                    cp.wait()
                for k, v in enumerate(hidden(NFC, NFC % 3, FREM, store_late)):
                    stab[k, 0:FREM // 2] = pltpu.bitcast(v, f32)
                db1[...] = db1s[:, 0:F].reshape(F).astype(bf16)
                for cp in cout(NFC - 2, (NFC - 2) % 3) + cout(NFC - 1, (NFC - 1) % 3):
                    cp.wait()

            wchunk = pltpu.VMEM((3, FC, S), bf16)
            pl.run_scoped(pass_hidden, wchunk, wchunk, pltpu.VMEM((1, S), f32),
                          pltpu.VMEM((1, S), f32), pltpu.SemaphoreType.DMA((2, 3)))

            def cout(t):
                return pltpu.make_async_copy(dob.at[_ds(t, TC)], out_hbm.at[_ds(t, TC)],
                                             osem.at[t])

            def pass_token(w1b, w2b, d1last, d2last, b2s, db2s, tsem, lsem):
                def cin(t):
                    s = t % 2
                    return (
                        pltpu.make_async_copy(w1T_hbm.at[:, _ds(t, TC)], w1b.at[s], tsem.at[0, s]),
                        pltpu.make_async_copy(w2_hbm.at[:, _ds(t, TC)], w2b.at[s], tsem.at[1, s]))

                start_now(*cin(0))
                d1last[...], d2last[...] = weight_grads(
                    *(_unpack(stab[k, 0:FREM // 2]) for k in range(2)))
                b2s[...] = b2[...].astype(f32).reshape(1, S)
                acc[...] = jnp.zeros(acc.shape, f32)
                clast = (pltpu.make_async_copy(d1last, dw1T_hbm.at[NFC * FC:], lsem.at[0]),
                         pltpu.make_async_copy(d2last, dw2_hbm.at[NFC * FC:], lsem.at[1]))
                for cp in clast:
                    cp.start()

                def transposed_pending():
                    words = jnp.concatenate(
                        [stab[1, 0:64, r:r + 128] for r in range(0, D, 128)], axis=0)
                    return _unpack(words).T

                def body(t, _):
                    @pl.when(t + 1 < NTC)
                    def _():
                        for cp in cin(t + 1):
                            cp.start()

                    for cp in cin(t):
                        cp.wait()
                    s = t % 2
                    always = zeros[...] == 0

                    def partial_sums(lhs, rhs):
                        sums = []
                        for ks in (slice(0, 512), slice(512, 1024), slice(1024, F)):
                            part = _dot(lhs[:, ks], rhs[ks])
                            sums.append(sums[-1] + part if sums else part)
                        return sums

                    def back(u, dh3, pace):
                        ts = _ds(u, 128)
                        doT = dob[ts, :].T.astype(f32)
                        x1 = load_panel(u, 128)
                        mu2, r2, mu3, r3 = (stats[i:i + 1, ts] for i in range(4))
                        xh2 = (_paced(x1, always, pace[0]) - mu2) * r2
                        xh3 = (xh2 * cols[2] + cols[1] - mu3) * r3
                        dh2 = _ln_bwd(dh3, xh3, r3, always, pace[1])
                        acc[0] += dh2
                        acc[1] += dh2 * xh2
                        store_panel(u, 128, doT + _ln_bwd(dh2 * cols[2], xh2, r2, always, pace[2]))
                        acc[2] += doT * b2s[:, _ds(u, 128)]
                        db2s[:, ts] = jnp.sum(cols[3] * doT, axis=0, keepdims=True)
                        return x1

                    def forth(u, y, x1):
                        return x1 + cols[3] * (y + b2s[:, _ds(u, 128)])

                    dh3 = [partial_sums(load_hidden(1), w1b[s, :, k:k + 128]) for k in (0, 128)]
                    y = [partial_sums(load_hidden(0), w2b[s, :, k:k + 128]) for k in (0, 128)]
                    first = back(2 * t, dh3[0][2], dh3[1])
                    second = back(2 * t + 1, dh3[1][2], y[0])
                    dob[_ds(jnp.maximum(2 * t - 1, 0), 128), :] = transposed_pending()
                    dob[_ds(2 * t, 128), :] = forth(2 * t, y[0][2], first).astype(bf16).T
                    words = pltpu.bitcast(forth(2 * t + 1, y[1][2], second).astype(bf16), f32)
                    for k in range(D // 128):
                        stab[1, 0:64, k * 128:(k + 1) * 128] = words[k * 64:(k + 1) * 64]

                    @pl.when(t > 0)
                    def _():
                        cout(t - 1).start()

                    return 0

                stab[1, 0:64] = jnp.zeros((64, QB), f32)
                lax.fori_loop(0, NTC, body, 0)
                dob[S - 128:] = transposed_pending()
                cout(NTC - 1).start()
                for k in range(3):
                    dmod[3 + k:4 + k] = _row_total(acc[k])
                dmod[5:6] += dmod[7:8]
                b2[...] = db2s[...].reshape(S).astype(bf16)
                for cp in clast:
                    cp.wait()

            wcols = pltpu.VMEM((2, F, TC), bf16)
            pl.run_scoped(pass_token, wcols, wcols, pltpu.VMEM((FREM, S), bf16),
                          pltpu.VMEM((FREM, S), bf16), pltpu.VMEM((1, S), f32),
                          pltpu.VMEM((1, S), f32), pltpu.SemaphoreType.DMA((2, 2)),
                          pltpu.SemaphoreType.DMA((2,)))

            def pass_project(wmhi, msem):
                cin, cgrad = mod_copies(wmhi, msem, 3)
                start_now(*cin)
                dmod[6:7] = jnp.zeros((1, D), f32)

                def project_back(j, dga, between=lambda: None):
                    ts = _ds(j, QB)
                    do = _dot(wsq[...], (load_panel(j, QB) * _wide(cols[0], QB)).astype(bf16))
                    between()
                    li = linv[:, ts]
                    do16 = jnp.concatenate(
                        [do[h * DH:(h + 1) * DH] * li[h:h + 1] for h in range(H)],
                        axis=0).astype(bf16)
                    prod = do16.astype(f32) * _unpack(oT[:, ts]).astype(f32)
                    linv[:, ts] = jnp.concatenate(
                        [jnp.sum(prod[h * DH:(h + 1) * DH], axis=0, keepdims=True)
                         for h in range(H)], axis=0)
                    aux[:, ts] = pltpu.bitcast(do16, i32)
                    dwo = _chain(jnp.add, [
                        _dot_nt(_unpack(oT[_ds(j, 64), _ds(k, QB)]), load_panel(k, QB).astype(bf16))
                        for k in range(S // QB)])
                    late[_ds(j, 64)] = _pack(dwo * mod[2:3])
                    return dga + jnp.sum(dwo * wsq[_ds(j, 128), :].astype(f32), axis=0, keepdims=True)

                def project_back_and_mod(j, dga):
                    def between():
                        dmod[6:7] += mod_grad(wmhi.at[j - 1], dmod[pl.ds(j + 2, 1)])

                    dga = project_back(j, dga, between)
                    cgrad(j - 1).start()
                    return dga

                kv = _unpack(kvT[...]).astype(f32)
                vk = _token_major(jnp.concatenate([kv[DH:], kv[:DH]], axis=0))
                is_v = lax.broadcasted_iota(i32, (1, 128), 1) < DH
                for c in range(NC):
                    ahead = (c + 1) % NC * KC
                    keys[_ds(c, KC // 2)] = _pack(jnp.concatenate(
                        [jnp.where(is_v, vk[c * KC:(c + 1) * KC - 16], 0.0),
                         jnp.where(is_v, 0.0, vk[ahead:ahead + 16])], axis=0))
                early[0, :, 0:128] = pltpu.bitcast(jnp.concatenate(
                    [vk[(c + 1) * KC - 16:(c + 1) * KC] for c in range(NC)], axis=0), i32)
                for c in range(NC // 2):
                    _spread_lanes(ltab, c, vk[(c + 1) * KC - 16:(c + 1) * KC])
                dga = project_back(0, jnp.zeros((1, D), f32))
                for cp in cin:
                    cp.wait()
                dmod[2:3] = lax.fori_loop(1, S // QB, project_back_and_mod, dga)
                wsq[...] = _unpack(late[0:D // 2])
                for c in range(NC // 2, NC):
                    _spread_lanes(ltab, c, pltpu.bitcast(early[0, _ds(c, 16), 0:128], f32))
                dwo_copy.start()
                for k in range(3):
                    cgrad(k).wait()

            pl.run_scoped(pass_project, pltpu.VMEM((3, D, D), bf16), pltpu.SemaphoreType.DMA((3,)))
            for t in range(NTC):
                cout(t).wait()

        pl.run_scoped(pass_mlp, pltpu.VMEM((2, D // 2, EARLY * FC), i32),
                      pltpu.SemaphoreType.DMA((NTC,)))

    pl.run_scoped(
        phase_main, pltpu.VMEM((D // 2, S), i32), pltpu.VMEM((S, D), bf16),
        pltpu.VMEM((S // 2, QB), i32), pltpu.SemaphoreType.DMA, pltpu.SemaphoreType.DMA)

    def phase_bwd(dkv, carried, xbuf, wmlo, sem, msem):
        cx = pltpu.make_async_copy(x_hbm, xbuf, sem.at[0])
        clo, cwlo = mod_copies(wmlo, msem, 0)

        def pass_attention_bwd():
            for cp in (*clo, cx):
                cp.start()
            dkv[...] = jnp.zeros_like(dkv)

            def spread(i, b):
                _spread_sublanes(stab.at[i % 2], _unpack(aux[_block(b)]))

            def query_row(ref, b):
                return jnp.broadcast_to(ref[pl.ds(b >> 2, 1), _block(b)[1]], (8, QB))

            def rows(x, n):
                return jnp.concatenate([x] * (n // 8), axis=0)

            def backward(blocks, slots):
                always = zeros[...] == 0
                ctx = [(aux[_block(b)], qT[_block(b)], query_row(linv, b), query_row(shift, b))
                       for b in blocks[:BBODY + 1]]
                first = carried[...]
                ds16, vpu = {}, {}
                dq = None
                n = BBODY * NC
                for t in range(n + 2):
                    tok = [None] * 8
                    if t + 1 < n:
                        i, c = divmod(t + 1, NC)
                        vpu[t + 1], tok = _vpu_dot(ltab, c, stab.at[i % 2],
                                                   rows(-ctx[i][2], 16), always)
                        if c == NC - 1:
                            spread(i, blocks[i + 2])
                    if t < n:
                        i, c = divmod(t, NC)
                        do, _, delta, _ = ctx[i]
                        words = [_after(x, tk, always) for x, tk in
                                 zip(key_groups(c, [7, *range(7)]),
                                     [None, None, tok[0], None] + tok[1:5])]
                        both = _dot(key_lhs(words, 2 * DH), _unpack(
                            jnp.concatenate([do, ctx[(t + 1) // NC][1]], axis=0)))
                        if t == 0:
                            vpu[0], _ = _vpu_dot(ltab, 0, stab.at[0],
                                                 rows(-delta, 16), always)
                        dp = jnp.concatenate([both[16:] - rows(delta, KC - 16), vpu.pop(t)], axis=0)
                        kept = _unpack(slots[i][_ds(c, KEPT), :])
                        p = jnp.concatenate([first, kept.astype(f32)], axis=0)
                        ds16[t] = (p * dp).astype(bf16)
                        dkv[DH:, _ds(c, KC)] += _dot_nt(_unpack(_after(do, tok[5], always)),
                                                        p.astype(bf16))
                        first = jnp.exp2(both[:16] - rows(ctx[(t + 1) // NC][3], 16))
                    if t >= 2:
                        i, c = divmod(t - 2, NC)
                        ds = ds16.pop(t - 2)
                        dkv[:DH, _ds(c, KC)] += _dot_nt(
                            _unpack(_after(ctx[i][1], tok[6], always)), ds)
                        part = _dot(_unpack(_after(kvT[0:8, _ds(c, KC)], tok[7], always)), ds)
                        dq = part if c == 0 else dq + part
                        if c == NC - 1:
                            qT[_block(blocks[i])] = _pack(dq * DH ** -0.5)
                carried[...] = first

            whole = NSLOT // BBODY

            def refills(n, action):
                @pl.when(jnp.logical_and(n >= 0, n < whole))
                def _():
                    action(fill_copy(NSPILL - (n + 1) * BBODY, BBODY))

                wrap = NSPILL - NSLOT
                for k in range(whole, pl.cdiv(NSPILL, BBODY)):
                    lo, hi = max(NSPILL - (k + 1) * BBODY, 0), NSPILL - k * BBODY

                    @pl.when(n == k)
                    def _():
                        for a, b in ((max(lo, wrap), hi), (lo, min(hi, wrap))):
                            if a < b:
                                action(fill_copy(a, b - a))

            def bwd_step(n, top):
                blocks = [NBLK - 1 - n * BBODY - i for i in range(BBODY + 2)]
                slots = [jnp.where(top < i, top - i + NSLOT, top - i) for i in range(BBODY + 1)]
                refills(n - whole, lambda cp: cp.wait())
                region(lambda: backward([jnp.maximum(b, 0) for b in blocks],
                                        [pool_slot(slot & 63) for slot in slots[:BBODY]]))
                refills(n, lambda cp: cp.start())

                @pl.when(n == 0)
                def _():
                    dwo_copy.wait()
                    wq_copy.start()

                return slots[BBODY]

            for i in range(2):
                spread(i, NBLK - 1 - i)
            q = qT[_block(NBLK - 1)]
            carried[...] = jnp.exp2(
                _dot(key_lhs(key_groups(NC - 1, [7]), 2 * DH),
                     _unpack(jnp.concatenate([jnp.zeros_like(q), q], axis=0)))
                - rows(query_row(shift, NBLK - 1), 16))
            lax.fori_loop(0, NBLK // BBODY, bwd_step, NSLOT - 1)

        pass_attention_bwd()

        def pass_qkv_bwd():
            cols, acc = ltab.at[2:4], ltab.at[0:2]
            cx.wait()
            wq_copy.wait()
            for cp in clo:
                cp.wait()
            cols[0] = _col(mod[0:1])
            cols[1] = _col(1.0 + mod[1:2])
            wkv = _token_major(jnp.concatenate(
                [wk[...], wv[...]], axis=0).astype(f32)).astype(bf16)
            kvT[...] = _pack(jnp.concatenate([dkv[:DH] * math.log(2.0), dkv[DH:]], axis=0))

            def dwq_share(j):
                ts = _ds(j, QB)
                part = _dot_nt(_unpack(aux[:, ts]), _unpack(qT[:, ts]))
                parts = [part[:, k * 128:(k + 1) * 128] for k in range(4)]
                return [v if j == 0 else ltab[4 + k] + v for k, v in enumerate(parts)]

            cdx = [pltpu.make_async_copy(xbuf.at[_ds(j, QB)], dx_hbm.at[_ds(j, QB)], sem.at[1 + j])
                   for j in range(S // QB)]
            for j in range(S // QB):
                always = zeros[...] == 0
                wqkv = jnp.concatenate([wsq[...], wkv], axis=1)[:, :D + 2 * DH]
                halves = range(j * QB // TC, (j + 1) * QB // TC)
                dhs = [_dot(wqkv, _unpack(jnp.concatenate(
                    [qT[:, _ds(t, TC)], kvT[:, _ds(t, TC)]], axis=0))) for t in halves]
                pace = [dhs[1], None]
                if j > 0:
                    for k, v in enumerate(dwq_share(j - 1)):
                        ltab[4 + k] = v
                        pace[1] = jnp.concatenate([v, v], axis=1) if k == 1 else pace[1]
                for t, dh, under in zip(halves, dhs, pace):
                    ts = _ds(t, TC)
                    ca_w = _wide(cols[1], TC)
                    _, r, xh = _ln_stats(xbuf[ts, :].T.astype(f32))
                    aux[:, ts] = _pack(xh * ca_w + _wide(cols[0], TC))
                    for k, v in enumerate((dh, dh * xh)):
                        acc[k] = _fold_lanes(v) if t == 0 else acc[k] + _fold_lanes(v)
                    dx = load_panel(t, TC) + _ln_bwd(dh * ca_w, xh, r, always, under)
                    xbuf[ts, :] = dx.astype(bf16).T
                if j == 0:
                    dmod[6:7] += mod_grad(wmlo.at[2], dmod[2:3])
                    start_now(cwlo(2))
                if j < S // QB - 1:
                    start_now(cdx[j])
            for k in range(2):
                dmod[k:k + 1] = _row_total(acc[k])
            dc = dmod[6:7] + mod_grad(wmlo.at[0], dmod[0:1]) + mod_grad(wmlo.at[1], dmod[1:2])
            c32 = cv[...].astype(f32)
            sig = jax.nn.sigmoid(c32)
            cv[...] = (dc * (sig * (1.0 + c32 * (1.0 - sig)))).astype(bf16)
            start_now(cwlo(0), cwlo(1), cdx[-1], *small_out[:3])
            wsq[...] = jnp.concatenate(dwq_share(S // QB - 1), axis=1).astype(bf16)
            dwq_copy = pltpu.make_async_copy(wsq, dwq_hbm, wsem)
            start_now(dwq_copy)
            dwkv = _dot_nt(_unpack(kvT[...]), _unpack(aux[...]))
            wk[...] = dwkv[:DH].astype(bf16)
            wv[...] = dwkv[DH:].astype(bf16)
            for cp in small_out[3:]:
                cp.start()
            for cp in (*map(cwlo, range(3)), *cdx, *small_out, dwq_copy):
                cp.wait()

        pass_qkv_bwd()

    pl.run_scoped(
        phase_bwd, pltpu.VMEM((2 * DH, S), f32), pltpu.VMEM((16, QB), f32), pltpu.VMEM((S, D), bf16),
        pltpu.VMEM((3, D, D), bf16), pltpu.SemaphoreType.DMA((5,)),
        pltpu.SemaphoreType.DMA((3,)))


@jax.jit
def pallas_adaLN_cond__grouped_kv_mqa__mixer_token_mlp__prompt_kernel(
    A_x: jax.Array,
    A_wq: jax.Array,
    A_wk: jax.Array,
    A_wv: jax.Array,
    A_wo: jax.Array,
    B_x: jax.Array,
    B_w1: jax.Array,
    B_b1: jax.Array,
    B_w2: jax.Array,
    B_b2: jax.Array,
    c: jax.Array,
    w_mod: jax.Array,
    grad_out: jax.Array,
):
    del B_x

    def sds(shape, dtype=bf16):
        return jax.ShapeDtypeStruct(shape, dtype)

    hbm = pl.BlockSpec(memory_space=pl.ANY)
    (dc, db1, db2, dwkT, dwvT, dx, dwq, dwo, dw1T, dw2, dwmod, out, _) = pl.pallas_call(
        _kernel,
        in_specs=[hbm] * 12,
        out_specs=[hbm] * 13,
        out_shape=[
            sds((1, D)), sds((F,)), sds((S,)), sds((DH, D)), sds((DH, D)), sds((S, D)),
            sds((D, D)), sds((D, D)), sds((F, S)), sds((F, S)), sds((D, 6 * D)), sds((S, D)),
            sds((NSPILL * SLOT, QB), i32),
        ],
        scratch_shapes=[
            pltpu.VMEM((NSLOT * SLOT + S, QB), i32),
            pltpu.VMEM((D // 2, S), i32),
            pltpu.VMEM((D // 2, S), i32),
            pltpu.VMEM((DH, S), i32),
            pltpu.VMEM((H, S), f32),
            pltpu.VMEM((H, S), f32),
            pltpu.VMEM((4, S), f32),
            pltpu.VMEM((8, D, 128), f32),
            pltpu.VMEM((2, 8 * DH, QB), f32),
            pltpu.VMEM((S // 2, 128), i32),
            pltpu.VMEM((8, D), f32),
            pltpu.VMEM((8, D), f32),
            pltpu.VMEM((8, 128), i32),
            pltpu.VMEM((D, D), bf16), pltpu.VMEM((DH, D), bf16), pltpu.VMEM((DH, D), bf16),
            pltpu.VMEM((S,), bf16), pltpu.VMEM((1, D), bf16),
            pltpu.VMEM((F,), bf16), pltpu.VMEM((F,), bf16),
            pltpu.SMEM((1,), i32),
            pltpu.SemaphoreType.DMA((NRING,)),
            pltpu.SemaphoreType.DMA,
            pltpu.SemaphoreType.DMA((5,)),
        ],
        compiler_params=pltpu.CompilerParams(
            vmem_limit_bytes=128 * 1024 * 1024, disable_bounds_checks=True),
        name="adaln_mqa_mixer_fwd_bwd",
    )(c, B_b1, B_b2, A_wk.T, A_wv.T,
      A_x.reshape(S, D), A_wq, A_wo, B_w1.T, B_w2, w_mod, grad_out.reshape(S, D))
    return (out.reshape(1, S, D), dx.reshape(1, S, D), dwq, dwkT.T, dwvT.T, dwo,
            dw1T.T, db1, dw2, db2, dc, dwmod)
```
